```python
import jax
import jax.numpy as jnp

def _softmax(x, axis=-1):
    return jax.nn.softmax(x, axis=axis)
def _gelu(x):
    return jax.nn.gelu(x, approximate=True)
def _silu(x):
    return jax.nn.silu(x)
def _sigmoid(x):
    return jax.nn.sigmoid(x)
def _layernorm(x, axis=-1, eps=1e-5):
    m = jnp.mean(x, axis=axis, keepdims=True)
    v = jnp.var(x, axis=axis, keepdims=True)
    return (x - m) / jnp.sqrt(v + eps)
def _scatter_add(tgt, idx, src, axis=0):
    return tgt.at[idx].add(src)
def _segment_sum(src, seg, n):
    return jax.ops.segment_sum(src, seg, n)
class _Rng:
    def __init__(self, key):
        self._k = key
    def _next(self):
        self._k, sub = jax.random.split(self._k)
        return sub
    def normal(self, shape):
        return jax.random.normal(self._next(), shape, dtype=jnp.bfloat16)
    def randint(self, lo, hi, shape):
        return jax.random.randint(self._next(), shape, lo, hi, dtype=jnp.int32)
    def uniform(self, shape, lo=0.0, hi=1.0):
        return jax.random.uniform(self._next(), shape, jnp.bfloat16, lo, hi)
    def permutation(self, n):
        return jax.random.permutation(self._next(), n)


kernel_name = 'sequential_preLN__grouped_kv_mqa__glu_gated_swiglu__prompt'

def _fwd_setup_inputs():
    _rng = _Rng(jax.random.key(int.from_bytes(__import__("os").urandom(4), "little")))
    _w = (lambda a: (lambda t: t.astype(jnp.bfloat16) if jnp.issubdtype(t.dtype, jnp.floating) else t)(jnp.asarray(a)))
    def _A_setup():
        B, S, D, H = 1, 2048, 512, 32
        Dh = D // H
        return {
            "x": _w((lambda *s: _rng.normal(s) * 0.05)(B, S, D)),
            "wq": _w((lambda *s: _rng.normal(s) * 0.05)(D, H * Dh)),
            "wk": _w((lambda *s: _rng.normal(s) * 0.05)(D, Dh)),
            "wv": _w((lambda *s: _rng.normal(s) * 0.05)(D, Dh)),
            "wo": _w((lambda *s: _rng.normal(s) * 0.05)(H * Dh, D)),
        }
    _A_in = _A_setup()

    def _B_setup():
        B, S, D, F = 1, 2048, 512, 1376
        return {
            "x": _w((lambda *s: _rng.normal(s) * 0.05)(B, S, D)),
            "w1": _w((lambda *s: _rng.normal(s) * 0.05)(D, F) * (2.0 / D) ** 0.5),
            "w3": _w((lambda *s: _rng.normal(s) * 0.05)(D, F) * (2.0 / D) ** 0.5),
            "w2": _w((lambda *s: _rng.normal(s) * 0.05)(F, D) * (2.0 / F) ** 0.5),
        }
    _B_in = _B_setup()

    return {
        "A_x": _A_in["x"],
        "A_wq": _A_in["wq"],
        "A_wk": _A_in["wk"],
        "A_wv": _A_in["wv"],
        "A_wo": _A_in["wo"],
        "B_x": _B_in["x"],
        "B_w1": _B_in["w1"],
        "B_w3": _B_in["w3"],
        "B_w2": _B_in["w2"],
    }

def _fwd_reference(A_x, A_wq, A_wk, A_wv, A_wo, B_x, B_w1, B_w3, B_w2):
    def _A_ref(x, wq, wk, wv, wo):
        B, S, D = x.shape
        H = 32
        Dh = D // H
        q = (lambda x, *d: x.transpose(*d))((x @ wq).reshape(B, S, H, Dh), 0, 2, 1, 3)
        k = x @ wk
        v = x @ wv
        scores = jnp.einsum("bhqd,bkd->bhqk", q, k) * (Dh ** -0.5)
        p = _softmax(scores, axis=-1)
        o = jnp.einsum("bhqk,bkd->bhqd", p, v)
        return (lambda x, *d: x.transpose(*d))(o, 0, 2, 1, 3).reshape(B, S, H * Dh) @ wo

    def _B_ref(x, w1, w3, w2):
        gate = jnp.einsum("bsd,df->bsf", x, w1)
        up = jnp.einsum("bsd,df->bsf", x, w3)
        h = _silu(gate) * up
        out = jnp.einsum("bsf,fd->bsd", h, w2)
        return out

    x = A_x
    h = x + _A_ref(_layernorm(x, axis=-1), A_wq, A_wk, A_wv, A_wo)
    h2 = h + _B_ref(_layernorm(h, axis=-1), B_w1, B_w3, B_w2)
    return h2


def setup_inputs():
    _inp = _fwd_setup_inputs()
    _gk = jax.random.fold_in(jax.random.key(int.from_bytes(__import__("os").urandom(4), "little")), 2**31 - 1)
    _shapes = [[1, 2048, 512]]
    _dtypes = ['bfloat16']
    _gks = jax.random.split(_gk, len(_shapes))
    _gs = [jax.random.normal(k, s, dtype=jnp.dtype(d)) * 0.05 for k, s, d in zip(_gks, _shapes, _dtypes)]
    _inp["grad_out"] = _gs[0]
    return _inp

def reference(A_x, A_wq, A_wk, A_wv, A_wo, B_w1, B_w3, B_w2, B_x, grad_out):
    _const = dict(B_x=B_x)
    def _f(*_d):
        return _fwd_reference(**{'A_x': _d[0], 'A_wq': _d[1], 'A_wk': _d[2], 'A_wv': _d[3], 'A_wo': _d[4], 'B_w1': _d[5], 'B_w3': _d[6], 'B_w2': _d[7], **_const})
    _out, _vjp = jax.vjp(_f, A_x, A_wq, A_wk, A_wv, A_wo, B_w1, B_w3, B_w2)
    _grads = _vjp(grad_out)
    _out0 = jnp.asarray(_out)
    return (_out0, *[jnp.asarray(_g) for _g in _grads])
```

```python
import jax
import jax.numpy as jnp
from jax import lax
import jax.experimental.pallas as pl
import jax.experimental.pallas.tpu as pltpu

S, D, H, DH, F = 2048, 512, 32, 16, 1376
BQ = 256
NT = BQ // 128
NC = S // 128
NB = S // BQ
G = NC // 2
UNF, LGF = 8, 3
UNB, LGB = 8, 2
FIN_UNROLL = 2
P0_UNROLL = 4
EPS = 1e-5
LOG2E = 1.4426950408889634
QSCALE = (DH ** -0.5) * LOG2E
SAFE_BOUND = 48.0
FCHUNKS = ((0, 512), (512, 512), (1024, 352))

f32, bf16 = jnp.float32, jnp.bfloat16
NTD = (((1,), (1,)), ((), ()))


def _dot(a, b):
    return jnp.dot(a, b, preferred_element_type=f32)


def _dot_nt(a, b):
    return lax.dot_general(a, b, NTD, preferred_element_type=f32)


def _ln_stats(x):
    mu = jnp.mean(x, axis=-1, keepdims=True)
    xc = x - mu
    var = jnp.mean(xc * xc, axis=-1, keepdims=True)
    rstd = lax.rsqrt(var + EPS)
    return xc * rstd, rstd


def _ln_bwd(dy, xhat, rstd):
    m1 = jnp.mean(dy, axis=-1, keepdims=True)
    m2 = jnp.mean(dy * xhat, axis=-1, keepdims=True)
    return rstd * (dy - m1 - xhat * m2)


def _split3(b):
    hi = b.astype(bf16).astype(f32)
    r1 = b - hi
    mid = r1.astype(bf16).astype(f32)
    lo = r1 - mid
    row = lax.broadcasted_iota(jnp.int32, (16, b.shape[1]), 0)
    t = jnp.where(row == 0, hi, jnp.where(row == 1, mid, jnp.where(row == 2, lo, 0.0)))
    return (-t).astype(bf16)


def _kernel(x_hbm, g_hbm, wq_hbm, wkT_hbm, wvT_hbm, wo_hbm, w1T_hbm, w3T_hbm, w2_hbm,
            out_hbm, dx_hbm, dwq_hbm, dwkT_hbm, dwvT_hbm, dwo_hbm, dw1T_hbm, dw3T_hbm, dw2_hbm,
            x_ref, g_ref, wq_ref, wkvT_ref, wo_ref, w1T_ref, w3T_ref, w2_ref,
            out_ref, dx_ref, dwq_ref, dwkvT_ref, dwo_ref, dw1T_ref, dw3T_ref, dw2_ref,
            xsem, gsem, wsem, osem,
            ln1_s, kext_s, v_s, kT_s, vT_s, wqT_s, qext_s, p_s, oT_s, linv_s, doT_s, delta_s,
            ds_s, dqT_s, dkv_s, dq_all, dh_all, dwo_a, dwqT_a, dw1_a, dw3_a, dw2T_a, acc_s, rstd_s):
    def blk(ref, b):
        return ref.at[pl.ds(pl.multiple_of(b * BQ, BQ), BQ)]

    def x_copy(b):
        return pltpu.make_async_copy(blk(x_hbm, b), blk(x_ref, b), xsem.at[b])

    def g_copy(b):
        return pltpu.make_async_copy(blk(g_hbm, b), blk(g_ref, b), gsem.at[b])

    w_copies = [
        pltpu.make_async_copy(wkT_hbm, wkvT_ref.at[0:16], wsem.at[0]),
        pltpu.make_async_copy(wvT_hbm, wkvT_ref.at[16:32], wsem.at[1]),
        pltpu.make_async_copy(wq_hbm, wq_ref, wsem.at[2]),
        pltpu.make_async_copy(wo_hbm, wo_ref, wsem.at[3]),
        pltpu.make_async_copy(w1T_hbm, w1T_ref, wsem.at[4]),
        pltpu.make_async_copy(w3T_hbm, w3T_ref, wsem.at[5]),
        pltpu.make_async_copy(w2_hbm, w2_ref, wsem.at[6]),
    ]
    x_copy(0).start()
    w_copies[0].start()
    w_copies[1].start()
    w_copies[2].start()
    for b in range(1, NB):
        x_copy(b).start()

    qext_s[NB * H] = jnp.zeros((NT, 32, 128), bf16)
    doT_s[H] = jnp.zeros((NT, 16, 128), bf16)
    delta_s[H] = jnp.zeros((NT, 1, 128), f32)
    dkv_s[...] = jnp.zeros_like(dkv_s)
    dwo_a[...] = jnp.zeros_like(dwo_a)
    dwqT_a[...] = jnp.zeros_like(dwqT_a)
    dw1_a[...] = jnp.zeros_like(dw1_a)
    dw3_a[...] = jnp.zeros_like(dw3_a)
    dw2T_a[...] = jnp.zeros_like(dw2T_a)
    w_copies[0].wait()
    w_copies[1].wait()

    w_copies[2].wait()
    wqT_s[...] = wq_ref[...].T
    for b in range(NB):
        x_copy(b).wait()
    for c in w_copies[3:]:
        c.start()
    for b in range(NB):
        g_copy(b).start()

    def ln1_blk(b, carry):
        kmax2, qmax2 = carry
        rows = pl.ds(pl.multiple_of(b * BQ, BQ), BQ)
        wkvT = wkvT_ref[...]
        xh, rstd = _ln_stats(x_ref[rows, :].astype(f32))
        rstd_s[rows, :] = jnp.broadcast_to(rstd, (BQ, 128))
        ln = xh.astype(bf16)
        ln1_s[rows, :] = ln
        kv = _dot_nt(ln, wkvT).astype(bf16)
        kvT = _dot_nt(wkvT, ln).astype(bf16)
        kext_s[rows, :] = kv
        v_s[rows, :] = kv[:, 16:32]
        kT_s[:, rows] = kvT[0:16]
        vT_s[:, rows] = kvT[16:32]
        kf = kvT[0:16].astype(f32)
        kmax2 = jnp.maximum(kmax2, jnp.sum(kf * kf, axis=0, keepdims=True))
        qb = (_dot_nt(wqT_s[...], ln) * QSCALE).astype(bf16)
        row = lax.broadcasted_iota(jnp.int32, (16, BQ), 0)
        for h in range(H):
            qh = qb[h * 16:(h + 1) * 16, :]
            qf = qh.astype(f32)
            n2 = jnp.sum(qf * qf, axis=0, keepdims=True)
            qmax2 = jnp.maximum(qmax2, n2)
            ext = jnp.where(row == 0, -jnp.sqrt(n2), 0.0).astype(bf16)
            for t in range(NT):
                qext_s[b * H + h, t, 0:16, :] = qh[:, t * 128:(t + 1) * 128]
                qext_s[b * H + h, t, 16:32, :] = ext[:, t * 128:(t + 1) * 128]
        return kmax2, qmax2

    kmax2, qmax2 = lax.fori_loop(0, NB, ln1_blk, (jnp.zeros((1, BQ), f32), jnp.zeros((1, BQ), f32)), unroll=P0_UNROLL)
    kmax2 = jnp.max(kmax2, axis=1, keepdims=True)
    qmax2 = jnp.max(qmax2, axis=1, keepdims=True)
    safe = jnp.max(kmax2 * qmax2) <= SAFE_BOUND * SAFE_BOUND
    lane = lax.broadcasted_iota(jnp.int32, (S, 32), 1)

    @pl.when(safe)
    def _bound():
        kmax = jnp.sqrt(kmax2).astype(bf16)
        kext_s[...] = jnp.where(lane < 16, kext_s[...], jnp.where(lane == 16, kmax, jnp.zeros_like(kmax)))

    @pl.when(jnp.logical_not(safe))
    def _true_max():
        kext_s[...] = jnp.where(lane < 16, kext_s[...], jnp.where(lane < 19, 1.0, 0.0).astype(bf16))

        def per_tile(i, c):
            h, t = i // NT, i % NT
            qe = qext_s[h, t, 0:16, :]

            def per_keys(kc, m):
                kk = kext_s[pl.ds(pl.multiple_of(kc * 128, 128), 128), 0:16]
                return jnp.maximum(m, jnp.max(_dot(kk, qe).reshape(16, 8, 128), axis=0))

            m = lax.fori_loop(0, NC, per_keys, jnp.full((8, 128), -jnp.inf, f32))
            qext_s[h, t, 16:32, :] = _split3(jnp.max(m, axis=0, keepdims=True))
            return c
        lax.fori_loop(0, NB * H * NT, per_tile, 0)

    o_copies = [
        pltpu.make_async_copy(dwo_ref, dwo_hbm, osem.at[1]),
        pltpu.make_async_copy(dw1T_ref, dw1T_hbm, osem.at[2]),
        pltpu.make_async_copy(dw3T_ref, dw3T_hbm, osem.at[3]),
        pltpu.make_async_copy(dw2_ref, dw2_hbm, osem.at[4]),
        pltpu.make_async_copy(dwq_ref, dwq_hbm, osem.at[5]),
        pltpu.make_async_copy(dwkvT_ref.at[0:16], dwkT_hbm, osem.at[6]),
        pltpu.make_async_copy(dwkvT_ref.at[16:32], dwvT_hbm, osem.at[7]),
    ]
    def w_out(j):
        if j == 0:
            dwkvT = jnp.zeros((32, D), f32)
            for c in range(NC):
                dkc = (dkv_s[0, c] * (1.0 / LOG2E)).astype(bf16)
                dvc = dkv_s[1, c].astype(bf16)
                dwkvT = dwkvT + _dot(jnp.concatenate([dkc, dvc], axis=0), ln1_s[c * 128:(c + 1) * 128, :])
            dwkvT_ref[...] = dwkvT.astype(dwkvT_ref.dtype)
            o_copies[5].start()
            o_copies[6].start()
        elif j == 1:
            dwo_ref[...] = dwo_a[...].astype(dwo_ref.dtype)
            o_copies[0].start()
        elif j == 2:
            dw1T_ref[...] = dw1_a[...].astype(bf16).T.astype(dw1T_ref.dtype)
            o_copies[1].start()
        elif j == 3:
            dw3T_ref[...] = dw3_a[...].astype(bf16).T.astype(dw3T_ref.dtype)
            o_copies[2].start()
        elif j == 4:
            dw2_ref[...] = dw2T_a[...].astype(bf16).T.astype(dw2_ref.dtype)
            o_copies[3].start()
        elif j == 5:
            dwq_ref[...] = dwqT_a[...].astype(bf16).T.astype(dwq_ref.dtype)
            o_copies[4].start()

    def s_group(pb, qe, u, g, l):
        for c in (2 * g, 2 * g + 1):
            for t in range(NT):
                p = jnp.exp2(_dot(kext_s[c * 128:(c + 1) * 128, :], qe[u, t]))
                lc = jnp.sum(p.reshape(16, 8, 128), axis=0)
                l[(u, t)] = lc if (u, t) not in l else l[(u, t)] + lc
                pb[u, t, c:c + 1] = p.reshape(1, 128, 128).astype(bf16)

    l0 = {}
    for g in range(LGF):
        s_group(p_s.at[pl.ds(H, 1)], qext_s, 0, g, l0)

    def block(b, lcar0):
        rows = pl.ds(pl.multiple_of(b * BQ, BQ), BQ)
        ln1 = ln1_s[rows, :]
        def pv_group(pb, ob, lb, u, g, acc, l):
            for c in (2 * g, 2 * g + 1):
                for t in range(NT):
                    a = _dot(vT_s[:, c * 128:(c + 1) * 128], pb[u, t, c])
                    acc[(u, t)] = a if (u, t) not in acc else acc[(u, t)] + a
                    if c == NC - 1:
                        linv = 1.0 / jnp.sum(l[(u, t)], axis=0, keepdims=True)
                        lb[u, t] = linv
                        ob[u * 16:(u + 1) * 16, t * 128:(t + 1) * 128] = acc[(u, t)] * linv

        def fwd_step(i, lcar):
            pb = p_s.at[pl.ds(i * UNF, UNF + 1)]
            qe = qext_s.at[pl.ds(b * H + i * UNF, UNF + 1)]
            lb = linv_s.at[pl.ds(i * UNF, UNF)]
            ob = oT_s.at[pl.ds(pl.multiple_of(i * UNF * 16, UNF * 16), UNF * 16)]
            l = {(0, t): lcar[t] for t in range(NT)}
            acc = {}
            for n in range(UNF * G):
                m = n + LGF
                s_group(pb, qe, m // G, m % G, l)
                pv_group(pb, ob, lb, n // G, n % G, acc, l)
            return tuple(l[(UNF, t)] for t in range(NT))

        p_s[0, :, 0:2 * LGF] = p_s[H, :, 0:2 * LGF]
        lcar1 = lax.fori_loop(0, H // UNF, fwd_step, lcar0)

        @pl.when(b == 0)
        def _():
            for c in w_copies[3:]:
                c.wait()
        g_copy(b).wait()
        gb = g_ref[rows, :]
        dacts = {0: _dot_nt(gb, w2_ref[0:FCHUNKS[0][1], :])}
        oTb = oT_s[...].astype(bf16)
        h1 = x_ref[rows, :].astype(f32) + _dot(oTb.T, wo_ref[...])
        xh2, rstd2 = _ln_stats(h1)
        ln2 = xh2.astype(bf16)
        ln2T = ln2.T
        gT = gb.T
        dacts[1] = _dot_nt(gb, w2_ref[FCHUNKS[1][0]:FCHUNKS[1][0] + FCHUNKS[1][1], :])
        acc_s[0] = h1
        acc_s[1] = jnp.zeros((BQ, D), f32)
        for ci, (f0, fc) in enumerate(FCHUNKS):
            fs = slice(f0, f0 + fc)
            dact = dacts[ci] if ci in dacts else _dot_nt(gb, w2_ref[fs, :])
            gate = _dot_nt(ln2, w1T_ref[fs, :])
            up = _dot_nt(ln2, w3T_ref[fs, :])
            sig = jax.nn.sigmoid(gate)
            silu = gate * sig
            act = (silu * up).astype(bf16)
            dup = (dact * silu).astype(bf16)
            dgate = (dact * up * (sig * (1.0 + gate * (1.0 - sig)))).astype(bf16)
            acc_s[0] += _dot(act, w2_ref[fs, :])
            acc_s[1] += _dot(dgate, w1T_ref[fs, :]) + _dot(dup, w3T_ref[fs, :])
            dw2T_a[:, fs] += _dot(gT, act)
            dw1_a[:, fs] += _dot(ln2T, dgate)
            dw3_a[:, fs] += _dot(ln2T, dup)
        out_ref[rows, :] = acc_s[0].astype(out_ref.dtype)
        pltpu.make_async_copy(blk(out_ref, b), blk(out_hbm, b), osem.at[0]).start()
        dh = gb.astype(f32) + _ln_bwd(acc_s[1], xh2, rstd2)
        dh_all[rows, :] = dh
        dhb = dh.astype(bf16)
        doT = _dot_nt(wo_ref[...], dhb)
        dwo_a[...] += _dot(oTb, dhb)
        for h in range(H):
            hs = slice(h * 16, (h + 1) * 16)
            for t in range(NT):
                ts = slice(t * 128, (t + 1) * 128)
                linv = linv_s[h, t]
                dob = (doT[hs, ts] * linv).astype(bf16)
                doT_s[h, t] = dob
                delta_s[h, t] = jnp.sum(dob.astype(f32) * oT_s[hs, ts], axis=0, keepdims=True)

        NS = 4 * (LGB + 2)

        def dp_group(pb, dob, deb, u, g, n):
            for j, c in enumerate((2 * g, 2 * g + 1)):
                for t in range(NT):
                    dp = _dot(v_s[c * 128:(c + 1) * 128, :], dob[u, t])
                    ds = pb[u, t, c].astype(f32) * (dp - deb[u, t])
                    ds_s[(n * 4 + j * 2 + t) % NS] = ds.astype(bf16)

        def small_group(pb, qe, dob, dqb, u, g, n, dq):
            units = [(j, c, t) for j, c in enumerate((2 * g, 2 * g + 1)) for t in range(NT)]
            a = {}
            for (j, c, t) in units:
                r = _dot_nt(qe[u, t, 0:16, :], ds_s[(n * 4 + j * 2 + t) % NS])
                a[j] = r if t == 0 else a[j] + r
                if t == NT - 1:
                    dkv_s[0, c] += a[j]
            for (j, c, t) in units:
                r = _dot_nt(dob[u, t], pb[u, t, c])
                a[j] = r if t == 0 else a[j] + r
                if t == NT - 1:
                    dkv_s[1, c] += a[j]
            for (j, c, t) in units:
                r = _dot(kT_s[:, c * 128:(c + 1) * 128], ds_s[(n * 4 + j * 2 + t) % NS])
                dq[(u, t)] = r if (u, t) not in dq else dq[(u, t)] + r
                if c == NC - 1:
                    dqb[u * 16:(u + 1) * 16, t * 128:(t + 1) * 128] = dq[(u, t)] * (DH ** -0.5)

        def bwd_step(i, c):
            pb = p_s.at[pl.ds(i * UNB, UNB + 1)]
            qe = qext_s.at[pl.ds(b * H + i * UNB, UNB + 1)]
            dob = doT_s.at[pl.ds(i * UNB, UNB + 1)]
            deb = delta_s.at[pl.ds(i * UNB, UNB + 1)]
            dqb = dqT_s.at[pl.ds(pl.multiple_of(i * UNB * 16, UNB * 16), UNB * 16)]
            dq = {}
            for n in range(UNB * G):
                m = n + LGB
                dp_group(pb, dob, deb, m // G, m % G, m)
                small_group(pb, qe, dob, dqb, n // G, n % G, n, dq)
            return c

        for g in range(LGB):
            dp_group(p_s, doT_s, delta_s, 0, g, g)
        lax.fori_loop(0, H // UNB, bwd_step, 0)

        dqTb = dqT_s[...].astype(bf16)
        dwqT_a[...] += _dot(dqTb, ln1)
        dq_all[rows, :] = dqTb.T
        return lcar1

    lax.fori_loop(0, NB, block, tuple(l0[(0, t)] for t in range(NT)))

    for j in (2, 3, 4, 1, 5, 0):
        w_out(j)

    def final_one(b):
        rows = pl.ds(pl.multiple_of(b * BQ, BQ), BQ)
        dln = _dot_nt(dq_all[rows, :], wq_ref[...])
        parts = []
        for cc in range(NT):
            c = b * NT + cc
            dkvT = jnp.concatenate([dkv_s[0, c] * (1.0 / LOG2E), dkv_s[1, c]], axis=0)
            parts.append(_dot(dkvT.astype(bf16).T, wkvT_ref[...]))
        dln = dln + jnp.concatenate(parts, axis=0)
        xh, rstd = ln1_s[rows, :].astype(f32), rstd_s[rows, 0:1]
        dx_ref[rows, :] = (dh_all[rows, :] + _ln_bwd(dln, xh, rstd)).astype(dx_ref.dtype)

    def final_blk(i, carry):
        for u in range(FIN_UNROLL):
            final_one(i * FIN_UNROLL + u)
        rows = pl.ds(pl.multiple_of(i * FIN_UNROLL * BQ, BQ), FIN_UNROLL * BQ)
        pltpu.make_async_copy(dx_ref.at[rows], dx_hbm.at[rows], osem.at[8]).start()
        return carry

    lax.fori_loop(0, NB // FIN_UNROLL, final_blk, 0)

    for c in o_copies:
        c.wait()
    pltpu.make_async_copy(out_ref, out_hbm, osem.at[0]).wait()
    pltpu.make_async_copy(dx_ref, dx_hbm, osem.at[8]).wait()


@jax.jit
def pallas_sequential_preLN__grouped_kv_mqa__glu_gated_swiglu__prompt_kernel(
    A_x: jax.Array,
    A_wq: jax.Array,
    A_wk: jax.Array,
    A_wv: jax.Array,
    A_wo: jax.Array,
    B_x: jax.Array,
    B_w1: jax.Array,
    B_w3: jax.Array,
    B_w2: jax.Array,
    grad_out: jax.Array,
):
    del B_x
    dt = A_x.dtype
    out_shape = (
        jax.ShapeDtypeStruct((S, D), dt), jax.ShapeDtypeStruct((S, D), dt),
        jax.ShapeDtypeStruct((D, D), dt), jax.ShapeDtypeStruct((DH, D), dt),
        jax.ShapeDtypeStruct((DH, D), dt), jax.ShapeDtypeStruct((D, D), dt),
        jax.ShapeDtypeStruct((F, D), dt), jax.ShapeDtypeStruct((F, D), dt),
        jax.ShapeDtypeStruct((F, D), dt),
    )
    scratch = [
        pltpu.VMEM((S, D), dt), pltpu.VMEM((S, D), dt), pltpu.VMEM((D, D), dt), pltpu.VMEM((32, D), dt),
        pltpu.VMEM((D, D), dt), pltpu.VMEM((F, D), dt), pltpu.VMEM((F, D), dt), pltpu.VMEM((F, D), dt),
        pltpu.VMEM((S, D), dt), pltpu.VMEM((S, D), dt), pltpu.VMEM((D, D), dt), pltpu.VMEM((32, D), dt),
        pltpu.VMEM((D, D), dt), pltpu.VMEM((F, D), dt), pltpu.VMEM((F, D), dt), pltpu.VMEM((F, D), dt),
        pltpu.SemaphoreType.DMA((NB,)), pltpu.SemaphoreType.DMA((NB,)),
        pltpu.SemaphoreType.DMA((7,)), pltpu.SemaphoreType.DMA((9,)),
        pltpu.VMEM((S, D), bf16),
        pltpu.VMEM((S, 32), bf16),
        pltpu.VMEM((S, 16), bf16),
        pltpu.VMEM((16, S), bf16),
        pltpu.VMEM((16, S), bf16),
        pltpu.VMEM((D, D), bf16),
        pltpu.VMEM((NB * H + 1, NT, 32, 128), bf16),
        pltpu.VMEM((H + 1, NT, NC, 128, 128), bf16),
        pltpu.VMEM((D, BQ), f32),
        pltpu.VMEM((H, NT, 1, 128), f32),
        pltpu.VMEM((H + 1, NT, 16, 128), bf16),
        pltpu.VMEM((H + 1, NT, 1, 128), f32),
        pltpu.VMEM((4 * (LGB + 2), 128, 128), bf16),
        pltpu.VMEM((D, BQ), f32),
        pltpu.VMEM((2, NC, 16, 128), f32),
        pltpu.VMEM((S, D), bf16),
        pltpu.VMEM((S, D), f32),
        pltpu.VMEM((D, D), f32),
        pltpu.VMEM((D, D), f32),
        pltpu.VMEM((D, F), f32),
        pltpu.VMEM((D, F), f32),
        pltpu.VMEM((D, F), f32),
        pltpu.VMEM((2, BQ, D), f32),
        pltpu.VMEM((S, 128), f32),
    ]
    outs = pl.pallas_call(
        _kernel,
        out_shape=out_shape,
        in_specs=[pl.BlockSpec(memory_space=pl.ANY)] * 9,
        out_specs=[pl.BlockSpec(memory_space=pl.ANY)] * 9,
        scratch_shapes=scratch,
        compiler_params=pltpu.CompilerParams(vmem_limit_bytes=110 * 1024 * 1024),
    )(A_x.reshape(S, D), grad_out.reshape(S, D), A_wq, A_wk.T, A_wv.T, A_wo, B_w1.T, B_w3.T, B_w2)
    out, dx, dwq, dwk, dwv, dwo, dw1, dw3, dw2 = outs
    return (out.reshape(1, S, D), dx.reshape(1, S, D), dwq, dwk.T, dwv.T, dwo, dw1.T, dw3.T, dw2)
```
